```python
import os as _os
_os.environ.setdefault("JAX_PLATFORMS", "cpu")
import jax
import jax.numpy as jnp

def _softmax(x, axis=-1):
    return jax.nn.softmax(x, axis=axis)
def _gelu(x):
    return jax.nn.gelu(x, approximate=True)
def _silu(x):
    return jax.nn.silu(x)
def _sigmoid(x):
    return jax.nn.sigmoid(x)
def _layernorm(x, axis=-1, eps=1e-5):
    m = jnp.mean(x, axis=axis, keepdims=True)
    v = jnp.var(x, axis=axis, keepdims=True)
    return (x - m) / jnp.sqrt(v + eps)
def _scatter_add(tgt, idx, src, axis=0):
    return tgt.at[idx].add(src)
def _segment_sum(src, seg, n):
    return jax.ops.segment_sum(src, seg, n)
class _Rng:
    def __init__(self, key):
        self._k = key
    def _next(self):
        self._k, sub = jax.random.split(self._k)
        return sub
    def normal(self, shape):
        return jax.random.normal(self._next(), shape, dtype=jnp.bfloat16)
    def randint(self, lo, hi, shape):
        return jax.random.randint(self._next(), shape, lo, hi, dtype=jnp.int32)
    def uniform(self, shape, lo=0.0, hi=1.0):
        return jax.random.uniform(self._next(), shape, jnp.bfloat16, lo, hi)
    def permutation(self, n):
        return jax.random.permutation(self._next(), n)


kernel_name = 'interleave_layers__linear_kernel_hedgehog__ssm_conv_s4__prompt'

def setup_inputs():
    _rng = _Rng(jax.random.key(int.from_bytes(__import__("os").urandom(4), "little")))
    _w = (lambda a: (lambda t: t.astype(jnp.bfloat16) if jnp.issubdtype(t.dtype, jnp.floating) else t)(jnp.asarray(a)))
    def _A_setup():
        B, S, D, H = 1, 2048, 512, 32
        Dh = D // H
        return {
            "x": _w((lambda *s: _rng.normal(s) * 0.05)(B, S, D)),
            "wqkv": _w((lambda *s: _rng.normal(s) * 0.4)(D, 3 * D)),
            "w_phi": _w((lambda *s: _rng.normal(s) * 0.4)(H, Dh, Dh) * (Dh ** -0.5)),
            "wo": _w((lambda *s: _rng.normal(s) * 0.05)(D, D)),
        }
    _A_in = _A_setup()

    def _B_setup():
        B, L, D, N = 1, 2048, 512, 128
        A_re = -jnp.exp((lambda *s: _rng.normal(s) * 0.2)(D, N))
        A_im = jnp.pi * (lambda *s: _rng.normal(s) * 0.2)(D, N)
        B_re = (lambda *s: _rng.normal(s) * 0.2)(D, N)
        B_im = (lambda *s: _rng.normal(s) * 0.2)(D, N)
        C_re = (lambda *s: _rng.normal(s) * 0.2)(D, N)
        C_im = (lambda *s: _rng.normal(s) * 0.2)(D, N)
        log_dt = (lambda *s: _rng.normal(s) * 0.2)(D) * 0.5 - 4.0
        Dskip = (lambda *s: _rng.normal(s) * 0.2)(D)
        return {
            "u": _w((lambda *s: _rng.normal(s) * 0.05)(B, L, D)),
            "A_re": _w(A_re),
            "A_im": _w(A_im),
            "B_re": _w(B_re),
            "B_im": _w(B_im),
            "C_re": _w(C_re),
            "C_im": _w(C_im),
            "log_dt": _w(log_dt),
            "Dskip": _w(Dskip),
        }
    _B_in = _B_setup()

    return {
        "A_x": _A_in["x"],
        "A_wqkv": _A_in["wqkv"],
        "A_w_phi": _A_in["w_phi"],
        "A_wo": _A_in["wo"],
        "B_u": _B_in["u"],
        "B_A_re": _B_in["A_re"],
        "B_A_im": _B_in["A_im"],
        "B_B_re": _B_in["B_re"],
        "B_B_im": _B_in["B_im"],
        "B_C_re": _B_in["C_re"],
        "B_C_im": _B_in["C_im"],
        "B_log_dt": _B_in["log_dt"],
        "B_Dskip": _B_in["Dskip"],
    }

def reference(A_x, A_wqkv, A_w_phi, A_wo, B_u, B_A_re, B_A_im, B_B_re, B_B_im, B_C_re, B_C_im, B_log_dt, B_Dskip):
    def _A_ref(x, wqkv, w_phi, wo):
        B, S, D = x.shape
        H = 32; Dh = D // H
        qkv = (lambda x, *d: x.transpose(*d))((x @ wqkv).reshape(B, S, 3, H, Dh), 2, 0, 3, 1, 4)
        q, k, v = qkv[0], qkv[1], qkv[2]
        pq = jnp.einsum("bhsd,hdf->bhsf", q, w_phi)
        pk = jnp.einsum("bhsd,hdf->bhsf", k, w_phi)
        phi_q = jnp.concatenate([_softmax(pq, axis=-1), _softmax(-pq, axis=-1)], axis=-1)
        phi_k = jnp.concatenate([_softmax(pk, axis=-1), _softmax(-pk, axis=-1)], axis=-1)
        kv = jnp.einsum("bhsf,bhsd->bhfd", phi_k, v)
        z  = jnp.einsum("bhsf->bhf", phi_k)
        num = jnp.einsum("bhqf,bhfd->bhqd", phi_q, kv)
        den = jnp.einsum("bhqf,bhf->bhq", phi_q, z)[..., None] + 1e-6
        o = num / den
        return (lambda x, *d: x.transpose(*d))(o, 0, 2, 1, 3).reshape(B, S, D) @ wo

    def _B_ref(u, A_re, A_im, B_re, B_im, C_re, C_im, log_dt, Dskip):
        Bsz, L, D = u.shape
        dt = jnp.exp(log_dt)[:, None]
        A = A_re + 1j * A_im
        Bc = B_re + 1j * B_im
        Cc = C_re + 1j * C_im
        logdA = dt * A
        dB = dt * Bc
        l = (lambda x, dt: x.astype(dt))(jnp.arange(L), A_re.dtype)
        P = jnp.exp(logdA[:, :, None] * l[None, None, :])
        K = jnp.einsum("dn,dnl,dn->dl", Cc, P, dB).real
        L2 = 2 * L
        Kp = jnp.pad(K, ((0, 0), (0, L)))
        up = (lambda x, *d: x.transpose(*d))(u, 0, 2, 1)
        up = jnp.pad(up, ((0, 0), (0, 0), (0, L)))
        Kf = (lambda x, axes=(-2,-1): jnp.fft.rfft2(x.astype(jnp.float32), axes=axes))(Kp[:, None, :], axes=(-2, -1))
        Uf = (lambda x, axes=(-2,-1): jnp.fft.rfft2(x.astype(jnp.float32), axes=axes))(up[:, :, None, :], axes=(-2, -1))
        Yf = Uf * Kf[None, :, :, :]
        y = (lambda x, s, axes=(-2,-1): jnp.fft.irfft2(x, s=s, axes=axes).astype(jnp.bfloat16))(Yf, (1, L2), axes=(-2, -1))[:, :, 0, :L]
        y = (lambda x, *d: x.transpose(*d))(y, 0, 2, 1) + u * Dskip[None, None, :]
        return y

    x = A_x
    x = x + _A_ref(_layernorm(x, axis=-1), A_wqkv, A_w_phi, A_wo)
    x = x + _B_ref(_layernorm(x, axis=-1), B_A_re, B_A_im, B_B_re, B_B_im, B_C_re, B_C_im, B_log_dt, B_Dskip)
    x = x + _A_ref(_layernorm(x, axis=-1), A_wqkv, A_w_phi, A_wo)
    x = x + _B_ref(_layernorm(x, axis=-1), B_A_re, B_A_im, B_B_re, B_B_im, B_C_re, B_C_im, B_log_dt, B_Dskip)
    return x
```

```python
import functools
import numpy as np
import jax
import jax.numpy as jnp
from jax import lax
import jax.experimental.pallas as pl
import jax.experimental.pallas.tpu as pltpu

S, D, H, DH, N = 2048, 512, 32, 16, 128
NB = S // 128
T = 512
NT = S // T
LOG2E = 1.4426950408889634
F32, BF16, U32 = jnp.float32, jnp.bfloat16, jnp.uint32


def _dft_consts():
    j = np.arange(128, dtype=np.float64)[:, None]
    k = np.arange(128, dtype=np.float64)[None, :]
    th = 2.0 * np.pi * j * (k + 0.5) / 256.0
    fwd = np.concatenate([np.cos(th), -np.sin(th)], axis=1)
    inv = np.concatenate([np.cos(th).T, -np.sin(th).T], axis=0) / 128
    return fwd.astype(np.float32), inv.astype(np.float32)


def _nt(a, b):
    return lax.dot_general(a, b, (((1,), (1,)), ((), ())), preferred_element_type=F32)


def _nn(a, b):
    return jnp.dot(a, b, preferred_element_type=F32)


def _cmul(ar, ai, br, bi):
    return ar * br - ai * bi, ar * bi + ai * br


def _csq(ar, ai):
    return ar * ar - ai * ai, (ar + ar) * ai


def _iota(shape, dim):
    return lax.broadcasted_iota(jnp.int32, shape, dim)


def _ldb(x):
    return pltpu.bitcast(x, BF16)


def _stb(x):
    return pltpu.bitcast(x.astype(BF16), U32)


def _kernel(x_hbm, wqkv_hbm, wphi_ref, wo_hbm, are_hbm, aim_hbm, bre_hbm, bim_hbm, cre_hbm, cim_hbm,
            ldt_ref, dsk_ref, ff_ref, fi_ref, o_hbm,
            xT, xn, wkv, wq, woT, kvacc, kvb, seed, mul, kt, t1, t2, t3, usta, ustb, ffs, fis,
            xin, wqkv_v, wo_v, par, ost, sems):
    par_cp = [pltpu.make_async_copy(src, par.at[i], sems.at[i])
              for i, src in enumerate((are_hbm, aim_hbm, bre_hbm, bim_hbm, cre_hbm, cim_hbm))]
    wqkv_cp = pltpu.make_async_copy(wqkv_hbm, wqkv_v, sems.at[6])
    x_cp = [pltpu.make_async_copy(x_hbm.at[pl.ds(i * T, T), :], xin.at[i], sems.at[7 + i]) for i in range(NT)]
    wo_cp = pltpu.make_async_copy(wo_hbm, wo_v, sems.at[7 + NT])
    for c in par_cp:
        c.start()
    wqkv_cp.start()
    for c in x_cp:
        c.start()
    wo_cp.start()

    r128, c128 = _iota((128, 128), 0), _iota((128, 128), 1)
    ones = jnp.ones((128, 128), BF16)
    ffs[...] = _stb(ff_ref[...])
    fis[...] = _stb(fi_ref[...])

    def col_bcast(row_ref, cb):
        v = jnp.broadcast_to(row_ref[:, cb * 128:(cb + 1) * 128], (128, 128))
        dg = jnp.where(r128 == c128, v.astype(F32), 0.0).astype(BF16)
        return _nn(dg, ones)

    for c in par_cp:
        c.wait()
    for cb in range(4):
        rows = slice(cb * 128, (cb + 1) * 128)
        dt = jnp.exp(col_bcast(ldt_ref, cb)).astype(BF16).astype(F32)
        al = dt * par[0, rows, :].astype(F32)
        be = dt * par[1, rows, :].astype(F32)
        mag = jnp.exp(al)
        l1r, l1i = mag * jnp.cos(be), mag * jnp.sin(be)
        br_, bi_ = dt * par[2, rows, :].astype(F32), dt * par[3, rows, :].astype(F32)
        wr, wi = _cmul(par[4, rows, :].astype(F32), par[5, rows, :].astype(F32), br_, bi_)
        pw = {1: (l1r, l1i)}
        p = 1
        while p < 1024:
            pw[2 * p] = _csq(*pw[p])
            p *= 2
        es = [(jnp.ones_like(l1r), jnp.zeros_like(l1r)), pw[1], pw[2]]
        es.append(_cmul(*pw[2], *pw[1]))
        es.append(pw[4])
        for s in range(1, 4):
            es.append(_cmul(*pw[4], *es[s]))
        ws = [(wr, wi)]
        ws.append(_cmul(wr, wi, *pw[128]))
        ws.append(_cmul(wr, wi, *pw[256]))
        ws.append(_cmul(*ws[1], *pw[256]))
        for s in range(4):
            ws.append(_cmul(*ws[s], *pw[512]))
        for s in range(8):
            for tb_, arr in enumerate((es[s][0], es[s][1], ws[s][0], -ws[s][1])):
                seed[tb_, cb * 16:(cb + 1) * 16, s * 8:(s + 1) * 8, :] = arr.reshape(16, 8, 128)
        for q, arr in enumerate((pw[8][0], pw[8][1], pw[64][0], -pw[64][1], pw[1024][0], -pw[1024][1])):
            mul[q, rows, :] = arr
        mul[6, rows, :] = col_bcast(dsk_ref, cb)

    hs_match = (r128 % 8) == (c128 // 16)
    perm = jnp.where(hs_match & ((r128 // 8) == (c128 % 16)), 1.0, 0.0).astype(BF16)
    rt = jnp.where((_iota((128, 16), 0) // 8) == _iota((128, 16), 1), 1.0, 0.0).astype(BF16)
    wqkv_cp.wait()
    for hb in range(4):
        w2 = wphi_ref[hb * 128:(hb + 1) * 128, :]
        bt = jnp.where(hs_match, _nt(rt, w2), 0.0).astype(BF16)
        wq[hb * 64:(hb + 1) * 64, :] = _stb(_nt(bt, wqkv_v[:, hb * 128:(hb + 1) * 128]) * LOG2E)
        wkv[hb * 128:hb * 128 + 64, :] = _stb(_nt(bt, wqkv_v[:, 512 + hb * 128:512 + (hb + 1) * 128]) * LOG2E)
        wkv[hb * 128 + 64:(hb + 1) * 128, :] = _stb(_nt(perm, wqkv_v[:, 1024 + hb * 128:1024 + (hb + 1) * 128]))
    for c in x_cp:
        c.wait()
    wo_cp.wait()
    for hb in range(4):
        wop = _nn(perm, wo_v[hb * 128:(hb + 1) * 128, :])
        woT[:, hb * 128:(hb + 1) * 128] = _stb(wop.T)

    lane_lo = c128[:8] < 64
    sgn = jnp.where((c128[:8] % 2) == 0, 1.0, -1.0).astype(F32)

    def kgen_pair(tile, sub0):
        lhs_r, lhs_i, rhs_r, rhs_i = [], [], [], []
        for c in range(2):
            sub = sub0 + c
            e_r, e_i, w_r, w_i = (seed[z, tile, pl.ds(sub, 8, stride=8), :] for z in range(4))
            m = [jnp.broadcast_to(mul[q, pl.ds(tile * 8 + sub, 1), :], (8, 128)) for q in range(6)]
            er, ei = [e_r], [e_i]
            for _s in range(7):
                a_, b_ = _cmul(er[-1], ei[-1], m[0], m[1])
                er.append(a_); ei.append(b_)
            w01 = _cmul(w_r, w_i, m[4], m[5])
            w10 = _cmul(w_r, w_i, m[2], m[3])
            w11 = _cmul(*w10, m[4], m[5])
            lhs_r.append(jnp.concatenate([w_r, w01[0], w10[0], w11[0]], axis=0))
            lhs_i.append(jnp.concatenate([w_i, w01[1], w10[1], w11[1]], axis=0))
            rhs_r.append(jnp.concatenate(er, axis=0))
            rhs_i.append(jnp.concatenate(ei, axis=0))
        lhs = jnp.concatenate([jnp.concatenate(lhs_r, axis=0), jnp.concatenate(lhs_i, axis=0)], axis=1).astype(BF16)
        rhs = jnp.concatenate([jnp.concatenate(rhs_r, axis=0), jnp.concatenate(rhs_i, axis=0)], axis=1).astype(BF16)
        o = _nt(lhs, rhs)
        for c in range(2):
            for mh in range(2):
                lo = o[c * 32 + mh * 8:c * 32 + mh * 8 + 8]
                hi = o[c * 32 + 16 + mh * 8:c * 32 + 16 + mh * 8 + 8]
                if c == 0:
                    v = jnp.where(lane_lo, lo, pltpu.roll(hi, 64, 1))
                else:
                    v = jnp.where(lane_lo, pltpu.roll(lo, 64, 1), hi)
                kt[pl.ds(pl.multiple_of(tile * 128 + (sub0 + c) * 16 + mh * 8, 8), 8), :] = v

    def ktab(ct):
        rows_ = [kt[pl.ds(ct * 128 + m, 8, stride=16), :] for m in range(16)]
        kf = _nn(jnp.concatenate(rows_, axis=0).astype(BF16), _ldb(ffs[...]))
        dsk = mul[6, pl.ds(pl.multiple_of(ct * 8, 8), 8), :]
        prev = None
        for m in range(16):
            cr, ci = kf[m * 8:(m + 1) * 8, :128], kf[m * 8:(m + 1) * 8, 128:]
            if m == 0:
                cr = cr + dsk
            if prev is None:
                wr_, wi_ = cr, ci
            else:
                wr_, wi_ = cr - sgn * prev[1], ci + sgn * prev[0]
            prev = (cr, ci)
            dst = pl.ds(pl.multiple_of(ct * 128 + m * 8, 8), 8)
            t1[dst, :] = wr_
            t2[dst, :] = wi_ - wr_
            t3[dst, :] = wi_ + wr_

    def layer_norm(xs):
        m = jnp.sum(xs, axis=0, keepdims=True) * (1.0 / D)
        xc = xs - m
        v = jnp.sum(xc * xc, axis=0, keepdims=True) * (1.0 / D)
        return (xc * lax.rsqrt(v + 1e-5)).astype(BF16)

    def feat(p):
        f = [p[i * 8:(i + 1) * 8] for i in range(16)]
        mx, mn = functools.reduce(jnp.maximum, f), functools.reduce(jnp.minimum, f)
        ep = [jnp.exp2(a - mx) for a in f]
        en = [jnp.exp2(mn - a) for a in f]
        rp = 1.0 / functools.reduce(jnp.add, ep)
        rn = 1.0 / functools.reduce(jnp.add, en)
        return jnp.concatenate([a * rp for a in ep] + [a * rn for a in en], axis=0).astype(BF16)

    TPB = (D // 8) // NT

    def pass1(first, tb, _):
        cols = pl.ds(pl.multiple_of(tb * T, T), T)
        if first:
            xs = jnp.concatenate(
                [jnp.concatenate([xin[tb, tt * 128:(tt + 1) * 128, cb * 128:(cb + 1) * 128].astype(F32).T
                                  for tt in range(T // 128)], axis=1) for cb in range(4)], axis=0)
            xT[:, cols] = xs
        else:
            xs = xT[:, cols]
        xb = layer_norm(xs)
        xn[:, cols] = pltpu.bitcast(xb, U32)
        kvall = _nn(_ldb(wkv[...]), xb)
        for hb in range(4):
            kv = kvall[hb * 256:(hb + 1) * 256]
            ph = feat(kv[:128])
            va = jnp.concatenate([kv[128:].astype(BF16), jnp.ones((16, T), BF16)], axis=0)
            kvacc[hb] += _nt(va, ph)
            if first:
                for t in range(hb * TPB // 4, (hb + 1) * TPB // 4):
                    for pr in range(4):
                        kgen_pair(tb * TPB + t, 2 * pr)
        return 0

    def pass2(first, tb, _):
        cols = pl.ds(pl.multiple_of(tb * T, T), T)
        xb = _ldb(xn[:, cols])
        qall = _nn(_ldb(wq[...]), xb)
        os_ = []
        for hb in range(4):
            ph = feat(qall[hb * 128:(hb + 1) * 128])
            nd = _nn(_ldb(kvb[hb]), ph)
            r = 1.0 / (nd[128:136] + 1e-6)
            os_.append(jnp.concatenate([nd[i * 8:(i + 1) * 8] * r for i in range(16)], axis=0).astype(BF16))
            if first:
                for t in range(hb * TPB // 4, (hb + 1) * TPB // 4):
                    ktab(tb * TPB + t)
        xnew = xT[:, cols] + _nn(_ldb(woT[...]), jnp.concatenate(os_, axis=0))
        xT[:, cols] = xnew
        xn[:, cols] = pltpu.bitcast(layer_norm(xnew), U32)
        return 0

    def layer_a(first):
        kvacc[...] = jnp.zeros_like(kvacc)
        lax.fori_loop(0, NT, functools.partial(pass1, first), 0)
        msk = (_iota((144, 256), 0) % 8) == (_iota((144, 256), 1) % 8)
        for hb in range(4):
            kvb[hb] = _stb(jnp.where(msk, kvacc[hb], 0.0))
        lax.fori_loop(0, NT, functools.partial(pass2, first), 0)

    def fwd(g, ub):
        u = jnp.concatenate([_ldb(xn[pl.ds(pl.multiple_of(g * 8, 8), 8), i * 128:(i + 1) * 128]) for i in range(NB)], axis=0)
        uf = _nn(u, _ldb(ffs[...]))
        for i in range(NB):
            for h in range(2):
                a, b = uf[i * 16 + h * 8:i * 16 + h * 8 + 8, :128], uf[i * 16 + h * 8:i * 16 + h * 8 + 8, 128:]
                ub[0, h, i * 8:(i + 1) * 8, :] = a
                ub[1, h, i * 8:(i + 1) * 8, :] = b
                ub[2, h, i * 8:(i + 1) * 8, :] = a + b

    def conv_inv(g, ub):
        for h in range(2):
            ct = g * 2 + h
            yr, yi = [], []
            for i in range(NB):
                k1 = k2 = k3 = None
                for m in range(i + 1):
                    base = pl.ds(pl.multiple_of(ct * 128 + m * 8, 8), 8)
                    c_, dm, dp = t1[base, :], t2[base, :], t3[base, :]
                    a, b, s_ = (ub[z, h, (i - m) * 8:(i - m + 1) * 8, :] for z in range(3))
                    if m == 0:
                        k1, k2, k3 = c_ * s_, a * dm, b * dp
                    else:
                        k1 += c_ * s_; k2 += a * dm; k3 += b * dp
                yr.append(k1 - k3); yi.append(k1 + k2)
            yv = jnp.concatenate([jnp.concatenate(yr, axis=0), jnp.concatenate(yi, axis=0)], axis=1).astype(BF16)
            y = _nn(yv, _ldb(fis[...]))
            rows8 = pl.ds(pl.multiple_of(ct * 8, 8), 8)
            for i in range(NB):
                xT[rows8, i * 128:(i + 1) * 128] += y[i * 8:(i + 1) * 8]

    NG = D // 16

    def b_body(g2, _):
        g = g2 * 2
        fwd(g + 1, ustb); conv_inv(g, usta)
        fwd(jnp.minimum(g + 2, NG - 1), usta); conv_inv(g + 1, ustb)
        return 0

    layer_a(True)
    fwd(0, usta)
    lax.fori_loop(0, NG // 2, b_body, 0)
    layer_a(False)
    fwd(0, usta)
    out_cp = []
    for cb in range(4):
        lax.fori_loop(cb * 4, cb * 4 + 4, b_body, 0)
        for tb in range(NB):
            ost[cb, tb * 128:(tb + 1) * 128, :] = \
                xT[cb * 128:(cb + 1) * 128, tb * 128:(tb + 1) * 128].T.astype(BF16)
        cp = pltpu.make_async_copy(ost.at[cb], o_hbm.at[:, pl.ds(cb * 128, 128)], sems.at[8 + NT + cb])
        cp.start()
        out_cp.append(cp)
    for cp in out_cp:
        cp.wait()


@jax.jit
def pallas_interleave_layers__linear_kernel_hedgehog__ssm_conv_s4__prompt_kernel(A_x, A_wqkv, A_w_phi, A_wo, B_u, B_A_re, B_A_im, B_B_re, B_B_im, B_C_re, B_C_im, B_log_dt, B_Dskip):
    ff, fi = _dft_consts()
    ff = jnp.asarray(ff, BF16); fi = jnp.asarray(fi, BF16)
    hbm = pl.BlockSpec(memory_space=pl.ANY)
    vm = pl.BlockSpec(memory_space=pltpu.VMEM)
    out = pl.pallas_call(
        _kernel,
        out_shape=jax.ShapeDtypeStruct((S, D), BF16),
        in_specs=[hbm, hbm, vm, hbm, hbm, hbm, hbm, hbm, hbm, hbm, vm, vm, vm, vm],
        out_specs=hbm,
        scratch_shapes=[
            pltpu.VMEM((D, S), F32), pltpu.VMEM((D // 2, S), U32),
            pltpu.VMEM((512, D), U32), pltpu.VMEM((256, D), U32), pltpu.VMEM((256, D), U32),
            pltpu.VMEM((4, 144, 256), F32), pltpu.VMEM((4, 72, 256), U32),
            pltpu.VMEM((4, 64, 64, 128), F32), pltpu.VMEM((7, D, 128), F32),
            pltpu.VMEM((D * 16, 128), F32),
            pltpu.VMEM((D * 16, 128), F32), pltpu.VMEM((D * 16, 128), F32), pltpu.VMEM((D * 16, 128), F32),
            pltpu.VMEM((3, 2, 128, 128), F32), pltpu.VMEM((3, 2, 128, 128), F32),
            pltpu.VMEM((64, 256), U32), pltpu.VMEM((128, 128), U32),
            pltpu.VMEM((NT, T, D), BF16), pltpu.VMEM((D, 3 * D), BF16), pltpu.VMEM((D, D), BF16),
            pltpu.VMEM((6, D, N), BF16), pltpu.VMEM((4, S, 128), BF16),
            pltpu.SemaphoreType.DMA((16,)),
        ],
        compiler_params=pltpu.CompilerParams(vmem_limit_bytes=100 * 1024 * 1024),
    )(A_x.reshape(S, D), A_wqkv, A_w_phi.reshape(H * DH, DH), A_wo, B_A_re, B_A_im, B_B_re, B_B_im, B_C_re, B_C_im,
      B_log_dt.reshape(1, D), B_Dskip.reshape(1, D), ff, fi)
    return out.reshape(1, S, D)
```

```python
import functools
import numpy as np
import jax
import jax.numpy as jnp
from jax import lax
import jax.experimental.pallas as pl
import jax.experimental.pallas.tpu as pltpu

S, D, H, DH, N = 2048, 512, 32, 16, 128
NB = S // 128
T = 512
NT = S // T
FRONT, LAG, BU = 16, 6, 4
T2F = 1024
T1S = 1024
T2S = 1024
LOG2E = 1.4426950408889634
F32, BF16, U32 = jnp.float32, jnp.bfloat16, jnp.uint32


def _dft_consts():
    j = np.arange(128, dtype=np.float64)[:, None]
    k = np.arange(128, dtype=np.float64)[None, :]
    th = 2.0 * np.pi * j * (k + 0.5) / 256.0
    fwd = np.concatenate([np.cos(th), -np.sin(th)], axis=1)
    inv = np.concatenate([np.cos(th).T, -np.sin(th).T], axis=0) / 128
    return fwd.astype(np.float32), inv.astype(np.float32)


def _nt(a, b):
    return lax.dot_general(a, b, (((1,), (1,)), ((), ())), preferred_element_type=F32)


def _nn(a, b):
    return jnp.dot(a, b, preferred_element_type=F32)


def _cmul(ar, ai, br, bi):
    return ar * br - ai * bi, ar * bi + ai * br


def _csq(ar, ai):
    return ar * ar - ai * ai, (ar + ar) * ai


def _cossin(x):
    k = jnp.floor(x * 0.6366197723675814 + 0.5)
    r = ((x - k * 1.5703125) - k * 4.837512969970703125e-4) - k * 7.54978995489188e-8
    z = r * r
    s_ = r + r * z * (-1.6666654611e-1 + z * (8.3321608736e-3 + z * -1.9515295891e-4))
    c_ = 1.0 - 0.5 * z + z * z * (4.166664568298827e-2 + z * (-1.388731625493765e-3 + z * 2.443315711809948e-5))
    q = k.astype(jnp.int32)
    odd = (q & 1) == 1
    sv, cv = jnp.where(odd, c_, s_), jnp.where(odd, s_, c_)
    sv = jnp.where((q & 2) == 2, -sv, sv)
    cv = jnp.where(((q + 1) & 2) == 2, -cv, cv)
    return cv, sv


def _iota(shape, dim):
    return lax.broadcasted_iota(jnp.int32, shape, dim)


def _ldb(x):
    return pltpu.bitcast(x, BF16)


def _stb(x):
    return pltpu.bitcast(x.astype(BF16), U32)


def _kernel(x_hbm, wqkv_hbm, wphi_ref, wo_hbm, are_hbm, aim_hbm, bre_hbm, bim_hbm, cre_hbm, cim_hbm,
            ldt_ref, dsk_ref, ff_ref, fi_ref, o_hbm,
            xT, xn, wkv, wq, woT, kvacc, kvb, seed, mul, kt, t1, t2, t3, usta, ustb, ffs, fis,
            xin, wqkv_v, wo_v, par, ost, sems):
    par_cp = [pltpu.make_async_copy(src, par.at[i], sems.at[i])
              for i, src in enumerate((are_hbm, aim_hbm, bre_hbm, bim_hbm, cre_hbm, cim_hbm))]
    wqkv_cp = pltpu.make_async_copy(wqkv_hbm, wqkv_v, sems.at[6])
    x_cp = [pltpu.make_async_copy(x_hbm.at[pl.ds(i * T, T), :], xin.at[i], sems.at[7 + i]) for i in range(NT)]
    wo_cp = pltpu.make_async_copy(wo_hbm, wo_v, sems.at[7 + NT])
    for c in par_cp:
        c.start()
    wqkv_cp.start()
    x_cp[0].start()
    wo_cp.start()
    for c in x_cp[1:]:
        c.start()

    r128, c128 = _iota((128, 128), 0), _iota((128, 128), 1)
    ones = jnp.ones((128, 128), BF16)
    ffs[...] = _stb(ff_ref[...])
    fis[...] = _stb(fi_ref[...])

    def col_bcast(row_ref, cb):
        v = jnp.broadcast_to(row_ref[...].astype(F32).reshape(1, D)[:, cb * 128:(cb + 1) * 128], (128, 128))
        dg = jnp.where(r128 == c128, v, 0.0).astype(BF16)
        return _nn(dg, ones)

    for cb in range(4):
        rows = slice(cb * 128, (cb + 1) * 128)
        mul[6, rows, :] = col_bcast(dsk_ref, cb)
        mul[7, rows, :] = jnp.exp(col_bcast(ldt_ref, cb)).astype(BF16).astype(F32)
    hs_match = ((r128 // 64) * 4 + r128 % 4) == (c128 // 16)
    perm = jnp.where(hs_match & (((r128 % 64) // 4) == (c128 % 16)), 1.0, 0.0).astype(BF16)
    rt = jnp.where(((_iota((128, 16), 0) % 64) // 4) == _iota((128, 16), 1), 1.0, 0.0).astype(BF16)
    us = [_nn(rt, wphi_ref[e]).astype(BF16) for e in range(DH)]
    hrow, ccol = _iota((H, D), 0), _iota((H, D), 1)
    acc = None
    for e in range(DH):
        sel = jnp.where((hrow == ccol // 16) & (ccol % 16 == e), 1.0, 0.0).astype(BF16)
        t_ = _nn(us[e], sel)
        acc = t_ if acc is None else acc + t_
    bts = [jnp.where(hs_match, acc[:, hb * 128:(hb + 1) * 128], 0.0).astype(BF16) for hb in range(4)]
    for c in par_cp:
        c.wait()
    CH = 64

    def seeds(it, _):
        rows = pl.ds(pl.multiple_of(it * CH, CH), CH)
        dt = mul[7, rows, :]
        al = dt * par[0, rows, :].astype(F32)
        be = dt * par[1, rows, :].astype(F32)
        mag = jnp.exp(al)
        cs, sn = _cossin(be)
        l1r, l1i = mag * cs, mag * sn
        br_, bi_ = dt * par[2, rows, :].astype(F32), dt * par[3, rows, :].astype(F32)
        wr, wi = _cmul(par[4, rows, :].astype(F32), par[5, rows, :].astype(F32), br_, bi_)
        tl = pl.ds(it * (CH // 8), CH // 8)

        def put(z, s, re, im):
            seed[z, tl, s * 8:(s + 1) * 8, :] = re.reshape(CH // 8, 8, 128)
            seed[z + 1, tl, s * 8:(s + 1) * 8, :] = im.reshape(CH // 8, 8, 128)

        p1 = (l1r, l1i)
        p2 = _csq(*p1)
        p4 = _csq(*p2)
        put(0, 0, jnp.ones_like(l1r), jnp.zeros_like(l1r))
        put(0, 1, *p1)
        put(0, 2, *p2)
        p3 = _cmul(*p2, *p1)
        put(0, 3, *p3)
        put(0, 4, *p4)
        put(0, 5, *_cmul(*p4, *p1))
        put(0, 6, *_cmul(*p4, *p2))
        put(0, 7, *_cmul(*p4, *p3))
        p8 = _csq(*p4)
        mul[0, rows, :] = p8[0]
        mul[1, rows, :] = p8[1]
        p64 = _csq(*_csq(*_csq(*p8)))
        mul[2, rows, :] = p64[0]
        mul[3, rows, :] = -p64[1]
        p128 = _csq(*p64)
        p256 = _csq(*p128)
        p512 = _csq(*p256)
        p1024 = _csq(*p512)
        mul[4, rows, :] = p1024[0]
        mul[5, rows, :] = -p1024[1]
        w0 = (wr, wi)
        w1 = _cmul(*w0, *p128)
        w2 = _cmul(*w0, *p256)
        w3 = _cmul(*w1, *p256)
        for s_, w_ in enumerate((w0, w1, w2, w3)):
            put(2, s_, w_[0], -w_[1])
            w4 = _cmul(*w_, *p512)
            put(2, s_ + 4, w4[0], -w4[1])
        return 0

    lax.fori_loop(0, D // CH, seeds, 0)

    wqkv_cp.wait()
    for hb in range(4):
        bt = bts[hb]
        wq[hb * 64:(hb + 1) * 64, :] = _stb(_nt(bt, wqkv_v[:, hb * 128:(hb + 1) * 128]) * LOG2E)
        wkv[hb * 128:hb * 128 + 64, :] = _stb(_nt(bt, wqkv_v[:, 512 + hb * 128:512 + (hb + 1) * 128]) * LOG2E)
        wkv[hb * 128 + 64:(hb + 1) * 128, :] = _stb(_nt(perm, wqkv_v[:, 1024 + hb * 128:1024 + (hb + 1) * 128]))
    wo_cp.wait()

    lane_lo = c128[:8] < 64
    sgn = jnp.where((c128[:8] % 2) == 0, 1.0, -1.0).astype(F32)

    def kgen_pair(tile, sub0):
        lhs_r, lhs_i, rhs_r, rhs_i = [], [], [], []
        for c in range(2):
            sub = sub0 + c
            e_r, e_i, w_r, w_i = (seed[z, tile, pl.ds(sub, 8, stride=8), :] for z in range(4))
            m = [jnp.broadcast_to(mul[q, pl.ds(tile * 8 + sub, 1), :], (8, 128)) for q in range(6)]
            er, ei = [e_r], [e_i]
            for _s in range(7):
                a_, b_ = _cmul(er[-1], ei[-1], m[0], m[1])
                er.append(a_); ei.append(b_)
            w01 = _cmul(w_r, w_i, m[4], m[5])
            w10 = _cmul(w_r, w_i, m[2], m[3])
            w11 = _cmul(*w10, m[4], m[5])
            lhs_r.append(jnp.concatenate([w_r, w01[0], w10[0], w11[0]], axis=0))
            lhs_i.append(jnp.concatenate([w_i, w01[1], w10[1], w11[1]], axis=0))
            rhs_r.append(jnp.concatenate(er, axis=0))
            rhs_i.append(jnp.concatenate(ei, axis=0))
        lhs = jnp.concatenate([jnp.concatenate(lhs_r, axis=0), jnp.concatenate(lhs_i, axis=0)], axis=1).astype(BF16)
        rhs = jnp.concatenate([jnp.concatenate(rhs_r, axis=0), jnp.concatenate(rhs_i, axis=0)], axis=1).astype(BF16)
        o = _nt(lhs, rhs)
        for c in range(2):
            for mh in range(2):
                lo = o[c * 32 + mh * 8:c * 32 + mh * 8 + 8]
                hi = o[c * 32 + 16 + mh * 8:c * 32 + 16 + mh * 8 + 8]
                if c == 0:
                    v = jnp.where(lane_lo, lo, pltpu.roll(hi, 64, 1))
                else:
                    v = jnp.where(lane_lo, pltpu.roll(lo, 64, 1), hi)
                kt[pl.ds(pl.multiple_of(tile * 128 + (sub0 + c) * 16 + mh * 8, 8), 8), :] = v

    def ktab(ct):
        rows_ = [kt[pl.ds(ct * 128 + m, 8, stride=16), :] for m in range(16)]
        kf = _nn(jnp.concatenate(rows_, axis=0).astype(BF16), _ldb(ffs[...]))
        dsk = mul[6, pl.ds(pl.multiple_of(ct * 8, 8), 8), :]
        prev = None
        for m in range(16):
            cr, ci = kf[m * 8:(m + 1) * 8, :128], kf[m * 8:(m + 1) * 8, 128:]
            if m == 0:
                cr = cr + dsk
            if prev is None:
                wr_, wi_ = cr, ci
            else:
                wr_, wi_ = cr - sgn * prev[1], ci + sgn * prev[0]
            prev = (cr, ci)
            dst = pl.ds(pl.multiple_of(ct * 128 + m * 8, 8), 8)
            t1[dst, :] = wr_
            t2[dst, :] = wi_ - wr_
            t3[dst, :] = wi_ + wr_

    def layer_norm(xs):
        m = jnp.sum(xs, axis=0, keepdims=True) * (1.0 / D)
        xc = xs - m
        v = jnp.sum(xc * xc, axis=0, keepdims=True) * (1.0 / D)
        return (xc * lax.rsqrt(v + 1e-5)).astype(BF16)

    def feat(p):
        f = [p[i * 8:(i + 1) * 8] for i in range(8)]
        mx, mn = functools.reduce(jnp.maximum, f), functools.reduce(jnp.minimum, f)
        mx = jnp.maximum(mx, pltpu.roll(mx, 4, 0))
        mn = jnp.minimum(mn, pltpu.roll(mn, 4, 0))
        ep = [jnp.exp2(a - mx) for a in f]
        en = [jnp.exp2(mn - a) for a in f]
        sp, sn = functools.reduce(jnp.add, ep), functools.reduce(jnp.add, en)
        rp = 1.0 / (sp + pltpu.roll(sp, 4, 0))
        rn = 1.0 / (sn + pltpu.roll(sn, 4, 0))
        return jnp.concatenate([a * rp for a in ep] + [a * rn for a in en], axis=0).astype(BF16)

    TPB = (D // 8) // NT

    def pass1(first, Tt, tb, _):
        cols = pl.ds(pl.multiple_of(tb * Tt, Tt), Tt)
        if first:
            pltpu.make_async_copy(x_hbm.at[pl.ds(pl.multiple_of(tb * T, T), T), :], xin.at[tb], sems.at[7 + tb]).wait()
            hcol = pl.ds(pl.multiple_of(tb * 128, 128), 128)
            wop = _nn(perm, wo_v[hcol, :])
            woT[:, hcol] = _stb(wop.T)
            for pp in range(FRONT):
                kgen_pair(tb * TPB + pp // 4, 2 * (pp % 4))
            xs = jnp.concatenate(
                [jnp.concatenate([xin[tb, tt * 128:(tt + 1) * 128, cb * 128:(cb + 1) * 128].astype(F32).T
                                  for tt in range(T // 128)], axis=1) for cb in range(4)], axis=0)
            xT[:, cols] = xs
        else:
            xs = xT[:, cols]
        xb = layer_norm(xs)
        xn[:, cols] = pltpu.bitcast(xb, U32)

        def kv_acc(hb, kv):
            for g2 in range(2):
                ph = feat(kv[g2 * 64:(g2 + 1) * 64])
                va = jnp.concatenate([kv[128 + g2 * 64:128 + (g2 + 1) * 64].astype(BF16),
                                      jnp.ones((16, Tt), BF16)], axis=0)
                kvacc[hb * 2 + g2] += _nt(va, ph)

        if first:
            parts = []
            rem = TPB * 4 - FRONT
            done = 0
            for di in range(16):
                parts.append(_nn(_ldb(wkv[di * 32:(di + 1) * 32, :]), xb))
                for pp in range(FRONT + di * rem // 16, FRONT + (di + 1) * rem // 16):
                    kgen_pair(tb * TPB + pp // 4, 2 * (pp % 4))
                while done < 4 and ((di + 1 - LAG) * 64 >= (done + 1) * 256 or di == 15):
                    kv_acc(done, jnp.concatenate(parts[done * 4:(done + 1) * 4], axis=0))
                    done += 1
        else:
            kvall = _nn(_ldb(wkv[...]), xb)
            for hb in range(4):
                kv_acc(hb, kvall[hb * 256:(hb + 1) * 256])
        return 0

    def pass2(first, Tt, tb, _):
        cols = pl.ds(pl.multiple_of(tb * Tt, Tt), Tt)
        tpb = (D // 8) // (S // Tt)
        xb = _ldb(xn[:, cols])
        qall = _nn(_ldb(wq[...]), xb)
        os_ = []
        for g in range(8):
            ph = feat(qall[g * 64:(g + 1) * 64])
            nd = _nn(_ldb(kvb[g]), ph)
            r = 1.0 / (nd[64:72] + 1e-6)
            os_.append(jnp.concatenate([nd[i * 8:(i + 1) * 8] * r for i in range(8)], axis=0).astype(BF16))
            if first:
                for t in range(g * tpb // 8, (g + 1) * tpb // 8):
                    ktab(tb * tpb + t)
        xnew = xT[:, cols] + _nn(_ldb(woT[...]), jnp.concatenate(os_, axis=0))
        xT[:, cols] = xnew
        xn[:, cols] = pltpu.bitcast(layer_norm(xnew), U32)
        return 0

    def layer_a(first, t1_, t2_):
        kvacc[...] = jnp.zeros_like(kvacc)
        lax.fori_loop(0, S // t1_, functools.partial(pass1, first, t1_), 0)
        msk = (_iota((80, 128), 0) % 4) == (_iota((80, 128), 1) % 4)
        for g in range(8):
            kvb[g] = _stb(jnp.where(msk, kvacc[g], 0.0))
        lax.fori_loop(0, S // t2_, functools.partial(pass2, first, t2_), 0)

    def fwd(g, ub):
        u = jnp.concatenate([_ldb(xn[pl.ds(pl.multiple_of(g * 8, 8), 8), i * 128:(i + 1) * 128]) for i in range(NB)], axis=0)
        uf = _nn(u, _ldb(ffs[...]))
        for i in range(NB):
            for h in range(2):
                a, b = uf[i * 16 + h * 8:i * 16 + h * 8 + 8, :128], uf[i * 16 + h * 8:i * 16 + h * 8 + 8, 128:]
                ub[0, h, i * 8:(i + 1) * 8, :] = a
                ub[1, h, i * 8:(i + 1) * 8, :] = b
                ub[2, h, i * 8:(i + 1) * 8, :] = a + b

    def conv_inv(g, ub):
        for h in range(2):
            ct = g * 2 + h
            yr, yi = [], []
            for i in range(NB):
                k1 = k2 = k3 = None
                for m in range(i + 1):
                    base = pl.ds(pl.multiple_of(ct * 128 + m * 8, 8), 8)
                    c_, dm, dp = t1[base, :], t2[base, :], t3[base, :]
                    a, b, s_ = (ub[z, h, (i - m) * 8:(i - m + 1) * 8, :] for z in range(3))
                    if m == 0:
                        k1, k2, k3 = c_ * s_, a * dm, b * dp
                    else:
                        k1 += c_ * s_; k2 += a * dm; k3 += b * dp
                yr.append(k1 - k3); yi.append(k1 + k2)
            yv = jnp.concatenate([jnp.concatenate(yr, axis=0), jnp.concatenate(yi, axis=0)], axis=1).astype(BF16)
            y = _nn(yv, _ldb(fis[...]))
            rows8 = pl.ds(pl.multiple_of(ct * 8, 8), 8)
            for i in range(NB):
                xT[rows8, i * 128:(i + 1) * 128] += y[i * 8:(i + 1) * 8]

    NG = D // 16

    GU = BU

    def out_block(cb):
        rows = pl.ds(pl.multiple_of(cb * 128, 128), 128)
        for tb in range(NB):
            ost[cb, tb * 128:(tb + 1) * 128, :] = xT[rows, tb * 128:(tb + 1) * 128].T.astype(BF16)

    def out_copy(cb):
        return pltpu.make_async_copy(ost.at[cb], o_hbm.at[:, pl.ds(pl.multiple_of(cb * 128, 128), 128)],
                                     sems.at[8 + NT + cb])

    def b_body(last, it, _):
        if last:
            out_block(jnp.maximum(it - 1, 0))
        for q in range(GU // 2):
            g = it * GU + 2 * q
            fwd(g + 1, ustb); conv_inv(g, usta)
            fwd(jnp.minimum(g + 2, NG - 1), usta); conv_inv(g + 1, ustb)
        if last:
            @pl.when(it > 0)
            def _():
                out_copy(it - 1).start()
        return 0

    layer_a(True, T, T2F)
    fwd(0, usta)
    lax.fori_loop(0, NG // GU, functools.partial(b_body, False), 0)
    layer_a(False, T1S, T2S)
    fwd(0, usta)
    GU = 8
    lax.fori_loop(0, NG // GU, functools.partial(b_body, True), 0)
    out_block(3)
    out_copy(3).start()
    for cb in range(4):
        out_copy(cb).wait()


@jax.jit
def pallas_interleave_layers__linear_kernel_hedgehog__ssm_conv_s4__prompt_kernel(A_x, A_wqkv, A_w_phi, A_wo, B_u, B_A_re, B_A_im, B_B_re, B_B_im, B_C_re, B_C_im, B_log_dt, B_Dskip):
    ff, fi = _dft_consts()
    ff = jnp.asarray(ff, BF16); fi = jnp.asarray(fi, BF16)
    hbm = pl.BlockSpec(memory_space=pl.ANY)
    vm = pl.BlockSpec(memory_space=pltpu.VMEM)
    out = pl.pallas_call(
        _kernel,
        out_shape=jax.ShapeDtypeStruct((S, D), BF16),
        in_specs=[hbm, hbm, vm, hbm, hbm, hbm, hbm, hbm, hbm, hbm, vm, vm, vm, vm],
        out_specs=hbm,
        scratch_shapes=[
            pltpu.VMEM((D, S), F32), pltpu.VMEM((D // 2, S), U32),
            pltpu.VMEM((512, D), U32), pltpu.VMEM((256, D), U32), pltpu.VMEM((256, D), U32),
            pltpu.VMEM((8, 80, 128), F32), pltpu.VMEM((8, 40, 128), U32),
            pltpu.VMEM((4, 64, 64, 128), F32), pltpu.VMEM((8, D, 128), F32),
            pltpu.VMEM((D * 16, 128), F32),
            pltpu.VMEM((D * 16, 128), F32), pltpu.VMEM((D * 16, 128), F32), pltpu.VMEM((D * 16, 128), F32),
            pltpu.VMEM((3, 2, 128, 128), F32), pltpu.VMEM((3, 2, 128, 128), F32),
            pltpu.VMEM((64, 256), U32), pltpu.VMEM((128, 128), U32),
            pltpu.VMEM((NT, T, D), BF16), pltpu.VMEM((D, 3 * D), BF16), pltpu.VMEM((D, D), BF16),
            pltpu.VMEM((6, D, N), BF16), pltpu.VMEM((4, S, 128), BF16),
            pltpu.SemaphoreType.DMA((16,)),
        ],
        compiler_params=pltpu.CompilerParams(vmem_limit_bytes=100 * 1024 * 1024),
    )(A_x.reshape(S, D), A_wqkv, jnp.transpose(A_w_phi, (1, 2, 0)), A_wo, B_A_re, B_A_im, B_B_re, B_B_im, B_C_re, B_C_im,
      B_log_dt, B_Dskip, ff, fi)
    return out.reshape(1, S, D)
```
